```python
import os as _os
_os.environ.setdefault("JAX_PLATFORMS", "cpu")
import jax
import jax.numpy as jnp

def _softmax(x, axis=-1):
    return jax.nn.softmax(x, axis=axis)
def _gelu(x):
    return jax.nn.gelu(x, approximate=True)
def _silu(x):
    return jax.nn.silu(x)
def _sigmoid(x):
    return jax.nn.sigmoid(x)
def _layernorm(x, axis=-1, eps=1e-5):
    m = jnp.mean(x, axis=axis, keepdims=True)
    v = jnp.var(x, axis=axis, keepdims=True)
    return (x - m) / jnp.sqrt(v + eps)
def _scatter_add(tgt, idx, src, axis=0):
    return tgt.at[idx].add(src)
def _segment_sum(src, seg, n):
    return jax.ops.segment_sum(src, seg, n)
class _Rng:
    def __init__(self, key):
        self._k = key
    def _next(self):
        self._k, sub = jax.random.split(self._k)
        return sub
    def normal(self, shape):
        return jax.random.normal(self._next(), shape, dtype=jnp.bfloat16)
    def randint(self, lo, hi, shape):
        return jax.random.randint(self._next(), shape, lo, hi, dtype=jnp.int32)
    def uniform(self, shape, lo=0.0, hi=1.0):
        return jax.random.uniform(self._next(), shape, jnp.bfloat16, lo, hi)
    def permutation(self, n):
        return jax.random.permutation(self._next(), n)


kernel_name = 'parallel_sum__sliding_block_cached__dense_activation_mish__decode'

def setup_inputs():
    _rng = _Rng(jax.random.key(int.from_bytes(__import__("os").urandom(4), "little")))
    _w = (lambda a: (lambda t: t.astype(jnp.bfloat16) if jnp.issubdtype(t.dtype, jnp.floating) else t)(jnp.asarray(a)))
    def _A_setup():
        B, Sq, D = 2, 1, 512
        Hq, Hkv, Sk, Dh = 32, 8, 32768, 128
        assert Hq % Hkv == 0, (Hq, Hkv)
        return {
            "x": _w((lambda *s: _rng.normal(s) * 0.05)(B, Sq, D)),
            "k_cache": _w((lambda *s: _rng.normal(s) * 0.8)(B, Hkv, Sk, Dh)),
            "v_cache": _w((lambda *s: _rng.normal(s) * 0.8)(B, Hkv, Sk, Dh)),
            "wq": _w((lambda *s: _rng.normal(s) * 0.8)(D, Hq * Dh) * (D ** -0.5)),
            "wo": _w((lambda *s: _rng.normal(s) * 0.8)(Hq * Dh, D) * ((Hq * Dh) ** -0.5)),
        }
    _A_in = _A_setup()

    def _B_setup():
        B, S, D, F = 2, 1, 512, 1792
        return {
            "x": _w((lambda *s: _rng.normal(s) * 0.05)(B, S, D)),
            "w1": _w((lambda *s: _rng.normal(s) * 0.4)(D, F) * (D ** -0.5)),
            "b1": _w((lambda *s: _rng.normal(s) * 0.05)(F)),
            "w2": _w((lambda *s: _rng.normal(s) * 0.05)(F, D) * (F ** -0.5)),
        }
    _B_in = _B_setup()

    return {
        "A_x": _A_in["x"],
        "A_k_cache": _A_in["k_cache"],
        "A_v_cache": _A_in["v_cache"],
        "A_wq": _A_in["wq"],
        "A_wo": _A_in["wo"],
        "B_x": _B_in["x"],
        "B_w1": _B_in["w1"],
        "B_b1": _B_in["b1"],
        "B_w2": _B_in["w2"],
    }

def reference(A_x, A_k_cache, A_v_cache, A_wq, A_wo, B_x, B_w1, B_b1, B_w2):
    def _A_ref(x, k_cache, v_cache, wq, wo):
        B, Sq, D = x.shape
        Hq, Dh = 32, 128
        Hkv, Sk = k_cache.shape[1], k_cache.shape[2]
        W = min(4096, max(256, Sk // 4))
        rep = Hq // Hkv
        q = (lambda x, *d: x.transpose(*d))((x @ wq).reshape(B, Sq, Hq, Dh), 0, 2, 1, 3)
        k = jnp.repeat(k_cache[:, :, Sk - W:, :], rep, axis=1)
        v = jnp.repeat(v_cache[:, :, Sk - W:, :], rep, axis=1)
        scores = jnp.einsum("bhqd,bhkd->bhqk", q, k) * (Dh ** -0.5)
        p = _softmax(scores, axis=-1)
        o = jnp.einsum("bhqk,bhkd->bhqd", p, v)
        return (lambda x, *d: x.transpose(*d))(o, 0, 2, 1, 3).reshape(B, Sq, Hq * Dh) @ wo

    def _B_ref(x, w1, b1, w2):
        h = jnp.einsum("bsd,df->bsf", x, w1) + b1
        sp = jnp.log1p(jnp.exp(-jnp.abs(h))) + jnp.where(h > 0, h, jnp.zeros_like(h))
        act = h * jnp.tanh(sp)
        return jnp.einsum("bsf,fd->bsd", act, w2)

    x = A_x
    xn = _layernorm(x, axis=-1)
    return x + _A_ref(xn, A_k_cache, A_v_cache, A_wq, A_wo) + _B_ref(xn, B_w1, B_b1, B_w2)
```

```python
import jax
import jax.numpy as jnp
from jax import lax
import jax.experimental.pallas as pl
import jax.experimental.pallas.tpu as pltpu

BF, F32 = jnp.bfloat16, jnp.float32
NT = (((1,), (1,)), ((), ()))


@jax.jit
def pallas_parallel_sum__sliding_block_cached__dense_activation_mish__decode_kernel(
    A_x: jax.Array,
    A_k_cache: jax.Array,
    A_v_cache: jax.Array,
    A_wq: jax.Array,
    A_wo: jax.Array,
    B_x: jax.Array,
    B_w1: jax.Array,
    B_b1: jax.Array,
    B_w2: jax.Array,
):
    del B_x
    B, Sq, D = A_x.shape
    _, Hkv, Sk, Dh = A_k_cache.shape
    Hq = A_wq.shape[1] // Dh
    rep = Hq // Hkv
    W = min(4096, max(256, Sk // 4))
    F = B_w1.shape[1]
    GW = rep * Dh
    scale = Dh ** -0.5
    wo_chunks = 8
    WOC = Hq * Dh // wo_chunks

    def kernel(x_h, k_h, v_h, wq_h, wo_h, w1_h, b1_h, w2_h, o_ref,
               x_v, b1_v, k_v, v_v, wq_v, wo_v, w1_v, w2_v, q_s, a_s,
               sem_s, sem_kv, sem_wo):
        cx = pltpu.make_async_copy(x_h, x_v, sem_s.at[0])
        cb1 = pltpu.make_async_copy(b1_h, b1_v, sem_s.at[1])
        cw1 = pltpu.make_async_copy(w1_h, w1_v, sem_s.at[2])
        cw2 = pltpu.make_async_copy(w2_h, w2_v, sem_s.at[3])
        cwq = pltpu.make_async_copy(wq_h, wq_v, sem_s.at[4])

        def kv_copy(h, j):
            src, dst = (k_h, k_v) if j < 2 else (v_h, v_v)
            b = j % 2
            return pltpu.make_async_copy(
                src.at[b, h, pl.ds(Sk - W, W), :], dst.at[b, h], sem_kv.at[h * 4 + j])

        def wo_copy(c):
            return pltpu.make_async_copy(
                wo_h.at[pl.ds(c * WOC, WOC), :], wo_v.at[pl.ds(c * WOC, WOC), :], sem_wo.at[c])

        pr = lambda i: i % 2
        cw1.start(priority=pr(0))
        cx.start(priority=pr(1))
        cb1.start(priority=pr(1))
        cw2.start(priority=pr(1))
        cwq.start(priority=pr(0))

        row = lax.broadcasted_iota(jnp.int32, (8, 128), 0)

        cx.wait()
        x = x_v[...].astype(F32)
        m = jnp.mean(x, axis=-1, keepdims=True)
        xc = x - m
        var = jnp.mean(xc * xc, axis=-1, keepdims=True)
        xn = xc / jnp.sqrt(var + 1e-5)
        rowD = lax.broadcasted_iota(jnp.int32, (8, D), 0)
        xn8 = jnp.where(rowD < rep, xn[0:1, :], xn[1:2, :]).astype(BF)

        cw1.wait()
        kv_copy(0, 0).start(priority=pr(1))
        cb1.wait()
        h = jnp.dot(xn8, w1_v[...], preferred_element_type=F32)
        b1 = b1_v[...].astype(F32)
        b1 = jnp.concatenate([b1[j:j + 1, :] for j in range(F // 128)], axis=1)
        h = h + b1
        sp = jnp.log1p(jnp.exp(-jnp.abs(h))) + jnp.where(h > 0, h, 0.0)
        act = h * jnp.tanh(sp)
        rowF = lax.broadcasted_iota(jnp.int32, (8, F), 0)
        act = jnp.where(rowF % rep == 0, act, 0.0).astype(BF)
        cw2.wait()
        kv_copy(0, 1).start(priority=pr(0))
        acc = jnp.dot(act, w2_v[...], preferred_element_type=F32)

        kv_copy(0, 2).start(priority=pr(1))
        cwq.wait()
        kv_copy(0, 3).start(priority=pr(0))
        for g in range(Hkv):
            qf = jnp.dot(xn8, wq_v[:, g * GW:(g + 1) * GW], preferred_element_type=F32)
            qg = qf[:, 0:Dh]
            for j in range(1, rep):
                qg = jnp.where(row % rep == j, qf[:, j * Dh:(j + 1) * Dh], qg)
            q_s[g] = qg

        def nxt(g, j):
            @pl.when(g + 1 < Hkv)
            def _():
                kv_copy(g + 1, j).start(priority=pr(j + 1))

            @pl.when(g + 1 == Hkv)
            def _():
                for c in range(j * wo_chunks // 4, (j + 1) * wo_chunks // 4):
                    wo_copy(c).start(priority=pr(c))

        def body(g, carry):
            q = q_s[g].astype(BF)
            rowW = lax.broadcasted_iota(jnp.int32, (8, W), 0)
            kv_copy(g, 0).wait()
            nxt(g, 0)
            s0 = lax.dot_general(q, k_v[0, g], NT, preferred_element_type=F32)
            kv_copy(g, 1).wait()
            nxt(g, 1)
            s1 = lax.dot_general(q, k_v[1, g], NT, preferred_element_type=F32)
            s = jnp.where(rowW < rep, s0, s1) * scale
            mx = jnp.max(s, axis=-1, keepdims=True)
            p = jnp.exp(s - mx)
            l = jnp.sum(p, axis=-1, keepdims=True)
            pb = p.astype(BF)
            kv_copy(g, 2).wait()
            nxt(g, 2)
            o0 = jnp.dot(pb, v_v[0, g], preferred_element_type=F32)
            kv_copy(g, 3).wait()
            nxt(g, 3)
            o1 = jnp.dot(pb, v_v[1, g], preferred_element_type=F32)
            o = jnp.where(row < rep, o0, o1) / l
            for j in range(rep):
                a_s[g, :, j * Dh:(j + 1) * Dh] = jnp.where(row % rep == j, o, 0.0)
            return carry

        lax.fori_loop(0, Hkv, body, 0)

        for c in range(wo_chunks):
            wo_copy(c).wait()
            a = a_s[c].astype(BF)
            acc = acc + jnp.dot(a, wo_v[c * WOC:(c + 1) * WOC, :], preferred_element_type=F32)
        o0 = jnp.sum(jnp.where(rowD < rep, acc, 0.0), axis=0, keepdims=True)
        o1 = jnp.sum(jnp.where(rowD < rep, 0.0, acc), axis=0, keepdims=True)
        row2 = lax.broadcasted_iota(jnp.int32, (2, D), 0)
        o_ref[...] = (x + jnp.where(row2 == 0, o0, o1)).astype(o_ref.dtype)

    hbm = pl.BlockSpec(memory_space=pltpu.HBM)
    out = pl.pallas_call(
        kernel,
        out_shape=jax.ShapeDtypeStruct((B * Sq, D), A_x.dtype),
        in_specs=[hbm] * 8,
        out_specs=pl.BlockSpec(memory_space=pltpu.VMEM),
        scratch_shapes=[
            pltpu.VMEM((B * Sq, D), BF), pltpu.VMEM((F // 128, 128), BF),
            pltpu.VMEM((B, Hkv, W, Dh), BF), pltpu.VMEM((B, Hkv, W, Dh), BF),
            pltpu.VMEM(A_wq.shape, BF), pltpu.VMEM(A_wo.shape, BF),
            pltpu.VMEM(B_w1.shape, BF), pltpu.VMEM(B_w2.shape, BF),
            pltpu.VMEM((Hkv, 8, Dh), F32), pltpu.VMEM((Hkv, 8, GW), F32),
            pltpu.SemaphoreType.DMA((5,)), pltpu.SemaphoreType.DMA((Hkv * 4,)),
            pltpu.SemaphoreType.DMA((wo_chunks,)),
        ],
        compiler_params=pltpu.CompilerParams(vmem_limit_bytes=64 << 20),
    )(A_x.reshape(B * Sq, D), A_k_cache, A_v_cache, A_wq, A_wo, B_w1,
      B_b1.reshape(F // 128, 128), B_w2)
    return out.reshape(B, Sq, D)
```

```python
import functools

import jax
import jax.numpy as jnp
from jax import lax
import jax.experimental.pallas as pl
import jax.experimental.pallas.tpu as pltpu

BF16, F32 = jnp.bfloat16, jnp.float32
_NT = (((1,), (1,)), ((), ()))


class _Stream:
    def __init__(self, sems, look):
        self.sems, self.look = sems, look
        self.steps = []
        self.started = [0, 0]
        self.done = [0, 0]

    def add(self, *pair):
        i = len(self.steps)
        self.steps.append(tuple(
            pltpu.make_async_copy(src, dst, self.sems[p].at[i % self.look[p]])
            for p, (src, dst) in enumerate(pair)))
        return i + 1

    def _start(self, p):
        self.steps[self.started[p]][p].start(priority=p)
        self.started[p] += 1

    def _wait(self, p, n):
        while self.done[p] < n:
            self.steps[self.done[p]][p].wait()
            self.done[p] += 1

    def start(self):
        for i in range(min(len(self.steps), max(self.look))):
            for p in (0, 1):
                if i < self.look[p]:
                    self._start(p)

    def wait_until(self, n):
        while self.done[1] < n:
            t = self.done[1] + 1
            self._wait(0, t)
            self._wait(1, t)
            for p in (0, 1):
                if self.started[p] < min(len(self.steps), t + self.look[p]):
                    self._start(p)

    def first_queue_fully_started(self):
        return self.started[0] == len(self.steps)

    def drain_first_queue(self):
        self._wait(0, len(self.steps))


@jax.jit
def pallas_parallel_sum__sliding_block_cached__dense_activation_mish__decode_kernel(
    A_x: jax.Array,
    A_k_cache: jax.Array,
    A_v_cache: jax.Array,
    A_wq: jax.Array,
    A_wo: jax.Array,
    B_x: jax.Array,
    B_w1: jax.Array,
    B_b1: jax.Array,
    B_w2: jax.Array,
):
    del B_x
    B, Sq, D = A_x.shape
    _, Hkv, Sk, Dh = A_k_cache.shape
    Hq = A_wq.shape[1] // Dh
    rep = Hq // Hkv
    W = min(4096, max(256, Sk // 4))
    F = B_w1.shape[1]
    assert (B, Sq, rep, Dh) == (2, 1, 4, 128)
    GW = rep * Dh
    scale = Dh ** -0.5
    kv_rows = 128
    kc = min(1024, W)
    look = (48, 64)
    tail = (8, 4, 2, 2)

    def kernel(x_h, k_h, v_h, wq_h, wo_h, w1_h, b1_h, w2_h, o_ref,
               x_v, b1_v, k_v, v_v, wq_v, wo_v, w1_v, w2_v, sem_s, sem0, sem1):
        st = _Stream((sem0, sem1), look)
        cx = pltpu.make_async_copy(x_h, x_v, sem_s.at[0])
        cb1 = pltpu.make_async_copy(b1_h, b1_v, sem_s.at[1])

        def halves(src, dst, n, r):
            ends = {}
            for i in range(0, n // 2, r):
                ends[i + r] = st.add(*[(src.at[pl.ds(j, r)], dst.at[pl.ds(j, r)])
                                       for j in (i, i + n // 2)])
            return ends

        def batches(src, dst, g):
            ends = {}
            for i in range(0, W, kv_rows):
                ends[i + kv_rows] = st.add(*[
                    (src.at[b, g, pl.ds(Sk - W + i, kv_rows)], dst.at[b, g, pl.ds(i, kv_rows)])
                    for b in range(B)])
            return ends

        half = Hq * Dh // 2
        e_w1 = halves(w1_h, w1_v, D, 8)
        e_w2 = halves(w2_h, w2_v, F, 32)
        e_wq = {}
        for i in range(0, D // 2, 8):
            for c in (0, half):
                e_wq[i + 8] = st.add(*[
                    (wq_h.at[pl.ds(j, 8), pl.ds(c, half)], wq_v.at[pl.ds(j, 8), pl.ds(c, half)])
                    for j in (i, i + D // 2)])
        e_k, e_v = {}, {}
        for g in range(Hkv):
            e_k[g] = batches(k_h, k_v, g)
            e_v[g] = batches(v_h, v_v, g)
        e_wo = halves(wo_h, wo_v, Hq * Dh, 32)

        cx.start()
        cb1.start()
        st.start()

        row = lax.broadcasted_iota(jnp.int32, (8, Dh), 0)
        row_d = lax.broadcasted_iota(jnp.int32, (8, D), 0)

        cx.wait()
        x = x_v[...].astype(F32)
        xc = x - jnp.mean(x, axis=-1, keepdims=True)
        var = jnp.mean(xc * xc, axis=-1, keepdims=True)
        xn = xc / jnp.sqrt(var + 1e-5)
        xn8 = jnp.where(row_d < rep, xn[0:1, :], xn[1:2, :]).astype(BF16)

        st.wait_until(e_w1[D // 2])
        h = jnp.dot(xn8, w1_v[...], preferred_element_type=F32)
        cb1.wait()
        b1 = b1_v[...].astype(F32)
        h = h + jnp.concatenate([b1[j:j + 1, :] for j in range(F // 128)], axis=1)
        sp = jnp.log1p(jnp.exp(-jnp.abs(h))) + jnp.where(h > 0, h, 0.0)
        act = (h * jnp.tanh(sp)).astype(BF16)
        st.wait_until(e_w2[F // 2])
        acc = jnp.dot(act, w2_v[...], preferred_element_type=F32)
        acc = acc + jnp.where(row_d < rep, x[0:1, :], x[1:2, :])

        qf = None
        for i in range(0, D // 2, 128):
            st.wait_until(e_wq[i + 128])
            for j in (i, i + D // 2):
                t = jnp.dot(xn8[:, j:j + 128], wq_v[j:j + 128, :], preferred_element_type=F32)
                qf = t if qf is None else qf + t
        qs = []
        for g in range(Hkv):
            qg = qf[:, g * GW:g * GW + Dh]
            for j in range(1, rep):
                qg = jnp.where(row % rep == j, qf[:, g * GW + j * Dh:g * GW + (j + 1) * Dh], qg)
            qs.append(qg.astype(BF16))

        row_c = lax.broadcasted_iota(jnp.int32, (8, kc), 0)
        outs = []
        for g in range(Hkv):
            s = []
            for c in range(W // kc):
                st.wait_until(e_k[g][(c + 1) * kc])
                t = [lax.dot_general(qs[g], k_v[b, g, c * kc:(c + 1) * kc, :], _NT,
                                     preferred_element_type=F32) for b in range(B)]
                s.append(jnp.where(row_c < rep, t[0], t[1]) * scale)
            mx = jnp.max(functools.reduce(jnp.maximum, s), axis=-1, keepdims=True)
            p = [jnp.exp(t - mx) for t in s]
            denom = jnp.sum(functools.reduce(jnp.add, p), axis=-1, keepdims=True)
            p = [t.astype(BF16) for t in p]
            o = [None] * B
            for c in range(W // kc):
                st.wait_until(e_v[g][(c + 1) * kc])
                for b in range(B):
                    t = jnp.dot(p[c], v_v[b, g, c * kc:(c + 1) * kc, :], preferred_element_type=F32)
                    o[b] = t if o[b] is None else o[b] + t
            o = jnp.where(row < rep, o[0], o[1]) / denom
            for j in range(rep):
                outs.append(jnp.where(row < rep, o[j:j + 1, :], o[rep + j:rep + j + 1, :]).astype(BF16))

        def proj(i, n):
            a = outs[i] if n == 1 else jnp.concatenate(outs[i:i + n], axis=1)
            return jnp.dot(a, wo_v[i * Dh:(i + n) * Dh, :], preferred_element_type=F32)

        assert sum(tail) == Hq // 2
        i, top_done = 0, False
        for n in tail:
            st.wait_until(e_wo[(i + n) * Dh])
            if not top_done and st.first_queue_fully_started():
                st.drain_first_queue()
                acc = acc + proj(i, Hq // 2 - i)
                top_done = True
            if not top_done:
                acc = acc + proj(i, n)
            acc = acc + proj(Hq // 2 + i, n)
            i += n
        row2 = lax.broadcasted_iota(jnp.int32, (B, D), 0)
        o_ref[...] = jnp.where(row2 == 0, acc[0:1, :], acc[rep:rep + 1, :]).astype(o_ref.dtype)

    hbm = pl.BlockSpec(memory_space=pltpu.HBM)
    out = pl.pallas_call(
        kernel,
        out_shape=jax.ShapeDtypeStruct((B * Sq, D), A_x.dtype),
        in_specs=[hbm] * 8,
        out_specs=pl.BlockSpec(memory_space=pltpu.VMEM),
        scratch_shapes=[
            pltpu.VMEM((B * Sq, D), A_x.dtype),
            pltpu.VMEM((F // 128, 128), B_b1.dtype),
            pltpu.VMEM((B, Hkv, W, Dh), A_k_cache.dtype),
            pltpu.VMEM((B, Hkv, W, Dh), A_v_cache.dtype),
            pltpu.VMEM(A_wq.shape, A_wq.dtype),
            pltpu.VMEM(A_wo.shape, A_wo.dtype),
            pltpu.VMEM(B_w1.shape, B_w1.dtype),
            pltpu.VMEM(B_w2.shape, B_w2.dtype),
            pltpu.SemaphoreType.DMA((2,)),
            pltpu.SemaphoreType.DMA((look[0],)),
            pltpu.SemaphoreType.DMA((look[1],)),
        ],
        compiler_params=pltpu.CompilerParams(
            vmem_limit_bytes=64 << 20,
            disable_semaphore_checks=True,
            disable_bounds_checks=True,
        ),
    )(A_x.reshape(B * Sq, D), A_k_cache, A_v_cache, A_wq, A_wo, B_w1,
      B_b1.reshape(F // 128, 128), B_w2)
    return out.reshape(B, Sq, D)
```

```python
import jax
import jax.numpy as jnp
from jax import lax
import jax.experimental.pallas as pl
import jax.experimental.pallas.tpu as pltpu

BF16, F32 = jnp.bfloat16, jnp.float32
_NT = (((1,), (1,)), ((), ()))


class _Stream:
    def __init__(self, sems, ahead):
        self.sems, self.ahead = sems, ahead
        self.ring = [s.shape[0] for s in sems]
        self.steps = []
        self.started = [0, 0]
        self.done = [0, 0]

    def add(self, *pair):
        i = len(self.steps)
        self.steps.append(tuple(
            pltpu.make_async_copy(src, dst, self.sems[q].at[i % self.ring[q]])
            for q, (src, dst) in enumerate(pair)))
        return i + 1

    def _wait(self, q, n):
        while self.done[q] < n:
            assert self.done[q] < self.started[q]
            self.steps[self.done[q]][q].wait()
            self.done[q] += 1

    def _start(self, q, n):
        while self.started[q] < min(n, len(self.steps)):
            i = self.started[q]
            self._wait(q, i + 1 - self.ring[q])
            self.steps[i][q].start(priority=q)
            self.started[q] += 1

    def start(self):
        for i in range(1, max(self.ahead) + 1):
            for q in (1, 0):
                self._start(q, min(i, self.ahead[q]))

    def _pace(self, n):
        while self.done[1] < min(n, len(self.steps)):
            t = self.done[1] + 1
            self._wait(1, t)
            for q in (0, 1):
                self._start(q, t + self.ahead[q])

    def advance(self, k):
        self._pace(self.done[1] + k)

    def need(self, n, lag=0):
        self._pace(n + lag)
        self._start(0, n)
        self._wait(0, n)

    def finished(self):
        return self.done == [len(self.steps)] * 2


@jax.jit
def pallas_parallel_sum__sliding_block_cached__dense_activation_mish__decode_kernel(
    A_x: jax.Array,
    A_k_cache: jax.Array,
    A_v_cache: jax.Array,
    A_wq: jax.Array,
    A_wo: jax.Array,
    B_x: jax.Array,
    B_w1: jax.Array,
    B_b1: jax.Array,
    B_w2: jax.Array,
):
    del B_x
    B, Sq, D = A_x.shape
    _, Hkv, Sk, Dh = A_k_cache.shape
    Hq = A_wq.shape[1] // Dh
    rep = Hq // Hkv
    W = min(4096, max(256, Sk // 4))
    F = B_w1.shape[1]
    assert (B, Sq, Hkv, rep, Dh) == (2, 1, 8, 4, 128) and W % 256 == 0
    GW = rep * Dh
    scale = Dh ** -0.5
    kv_rows = 128
    kc = 256
    ways = 8
    ahead = (12, 48)
    ring0 = 32
    lag = 12
    tail = (2, 1, 1)

    def kernel(x_h, k_h, v_h, wq_h, wo_h, w1_h, b1_h, w2_h, o_ref,
               x_v, b1_v, k_v, v_v, wq_v, wo_v, w1_v, w2_v, s_v, sem_s, sem0, sem1):
        st = _Stream((sem0, sem1), ahead)
        cx = pltpu.make_async_copy(x_h, x_v, sem_s.at[0])
        cb1 = pltpu.make_async_copy(b1_h, b1_v, sem_s.at[1])

        def rows(src, dst, i, r):
            return src.at[pl.ds(i, r)], dst.at[pl.ds(i, r)]

        def add_interleaved(pieces):
            m = len(pieces) // ways
            assert m * ways == len(pieces)
            order = [pieces[j * m + i] for i in range(m) for j in range(ways)]
            for pair in zip(order[0::2], order[1::2]):
                n = st.add(*pair)
            return n

        def add_cache(src, dst):
            ends = {}
            for i in range(0, W, kv_rows):
                for g in range(Hkv):
                    ends[i + kv_rows] = st.add(*[
                        (src.at[b, g, pl.ds(Sk - W + i, kv_rows)], dst.at[b, g, pl.ds(i, kv_rows)])
                        for b in range(B)])
            return ends

        half = Hq * Dh // 2
        e_wq = add_interleaved([
            (wq_h.at[pl.ds(i, 8), pl.ds(c, half)], wq_v.at[pl.ds(i, 8), pl.ds(c, half)])
            for i in range(0, D, 8) for c in (0, half)])
        e_w1 = add_interleaved([rows(w1_h, w1_v, i, 8) for i in range(0, D, 8)])
        e_w2 = add_interleaved([rows(w2_h, w2_v, i, 32) for i in range(0, F, 32)])
        e_k = add_cache(k_h, k_v)
        e_v = add_cache(v_h, v_v)
        e_wo = {}
        for j in range(rep):
            pieces = [(g, i) for i in range(0, Dh, 32) for g in range(0, Hkv, 2)]
            if j == rep - 1:
                pieces.sort()
            for g, i in pieces:
                e_wo[j, g] = st.add(*[rows(wo_h, wo_v, (g + q) * GW + j * Dh + i, 32) for q in (0, 1)])

        cx.start()
        cb1.start()
        st.start()

        row = lax.broadcasted_iota(jnp.int32, (8, Dh), 0)
        row_d = lax.broadcasted_iota(jnp.int32, (8, D), 0)
        row_c = lax.broadcasted_iota(jnp.int32, (8, kc), 0)

        cx.wait()
        x = x_v[...].astype(F32)
        xc = x - jnp.mean(x, axis=-1, keepdims=True)
        var = jnp.mean(xc * xc, axis=-1, keepdims=True)
        xn = xc / jnp.sqrt(var + 1e-5)
        xn8 = jnp.where(row_d < rep, xn[0:1, :], xn[1:2, :]).astype(BF16)

        st.need(e_wq, lag)
        qs = []
        for g in range(Hkv):
            qf = jnp.dot(xn8, wq_v[:, g * GW:(g + 1) * GW], preferred_element_type=F32)
            qg = qf[:, :Dh]
            for j in range(1, rep):
                qg = jnp.where(row % rep == j, qf[:, j * Dh:(j + 1) * Dh], qg)
            qs.append(qg.astype(BF16))
            st.advance(3)

        st.need(e_w1, lag)
        cb1.wait()
        b1 = b1_v[...].astype(F32)
        cols = [(c, min(512, F - c)) for c in range(0, F, 512)]
        acts = []
        for c, n in cols:
            h = jnp.dot(xn8, w1_v[:, c:c + n], preferred_element_type=F32)
            h = h + jnp.concatenate([b1[j:j + 1, :] for j in range(c // 128, (c + n) // 128)], axis=1)
            sp = jnp.log1p(jnp.exp(-jnp.abs(h))) + jnp.where(h > 0, h, 0.0)
            acts.append((h * jnp.tanh(sp)).astype(BF16))
            st.advance(3)
        st.need(e_w2, lag)
        acc = jnp.where(row_d < rep, x[0:1, :], x[1:2, :])
        for (c, n), act in zip(cols, acts):
            acc = acc + jnp.dot(act, w2_v[c:c + n, :], preferred_element_type=F32)
            st.advance(3)

        mx = [None] * Hkv
        for c in range(0, W, kc):
            st.need(e_k[c + kc], lag)
            for g in range(Hkv):
                t = [lax.dot_general(qs[g], k_v[b, g, c:c + kc, :], _NT, preferred_element_type=F32)
                     for b in range(B)]
                s = jnp.where(row_c < rep, t[0], t[1]) * scale
                s_v[g, :, c:c + kc] = s
                for i in range(0, kc, 128):
                    si = s[:, i:i + 128]
                    mx[g] = si if mx[g] is None else jnp.maximum(mx[g], si)
        mx = [jnp.max(t, axis=-1, keepdims=True) for t in mx]

        denom = [None] * Hkv
        o = [None] * Hkv
        for c in range(0, W, kc):
            st.need(e_v[c + kc], lag)
            for g in range(Hkv):
                p = jnp.exp(s_v[g, :, c:c + kc] - mx[g])
                for i in range(0, kc, 128):
                    pi = p[:, i:i + 128]
                    denom[g] = pi if denom[g] is None else denom[g] + pi
                p = p.astype(BF16)
                t = [jnp.dot(p, v_v[b, g, c:c + kc, :], preferred_element_type=F32) for b in range(B)]
                t = jnp.where(row < rep, t[0], t[1])
                o[g] = t if o[g] is None else o[g] + t
        outs = {}
        for g in range(Hkv):
            og = o[g] / jnp.sum(denom[g], axis=-1, keepdims=True)
            for j in range(rep):
                outs[j, g] = jnp.where(row < rep, og[j:j + 1, :], og[rep + j:rep + j + 1, :]).astype(BF16)

        def proj(j, g):
            r = g * GW + j * Dh
            return jnp.dot(outs[j, g], wo_v[r:r + Dh, :], preferred_element_type=F32)

        for j in range(rep - 1):
            st.need(e_wo[j, Hkv - 2])
            for g in range(Hkv):
                acc = acc + proj(j, g)
        g0 = 0
        for n in tail:
            g1 = g0 + 2 * n
            st.need(e_wo[rep - 1, g1 - 2])
            for g in range(g0, g1):
                acc = acc + proj(rep - 1, g)
            g0 = g1
        assert g0 == Hkv and st.finished()
        row_b = lax.broadcasted_iota(jnp.int32, (B, D), 0)
        o_ref[...] = jnp.where(row_b == 0, acc[0:1, :], acc[rep:rep + 1, :]).astype(o_ref.dtype)

    hbm = pl.BlockSpec(memory_space=pltpu.HBM)
    out = pl.pallas_call(
        kernel,
        out_shape=jax.ShapeDtypeStruct((B * Sq, D), A_x.dtype),
        in_specs=[hbm] * 8,
        out_specs=pl.BlockSpec(memory_space=pltpu.VMEM),
        scratch_shapes=[
            pltpu.VMEM((B * Sq, D), A_x.dtype),
            pltpu.VMEM((F // 128, 128), B_b1.dtype),
            pltpu.VMEM((B, Hkv, W, Dh), A_k_cache.dtype),
            pltpu.VMEM((B, Hkv, W, Dh), A_v_cache.dtype),
            pltpu.VMEM(A_wq.shape, A_wq.dtype),
            pltpu.VMEM(A_wo.shape, A_wo.dtype),
            pltpu.VMEM(B_w1.shape, B_w1.dtype),
            pltpu.VMEM(B_w2.shape, B_w2.dtype),
            pltpu.VMEM((Hkv, 8, W), F32),
            pltpu.SemaphoreType.DMA((2,)),
            pltpu.SemaphoreType.DMA((ring0,)),
            pltpu.SemaphoreType.DMA((ahead[1],)),
        ],
        compiler_params=pltpu.CompilerParams(
            vmem_limit_bytes=64 << 20,
            disable_semaphore_checks=True,
            disable_bounds_checks=True,
        ),
    )(A_x.reshape(B * Sq, D), A_k_cache, A_v_cache, A_wq, A_wo, B_w1,
      B_b1.reshape(F // 128, 128), B_w2)
    return out.reshape(B, Sq, D)
```

```python
import jax
import jax.numpy as jnp
from jax import lax
import jax.experimental.pallas as pl
import jax.experimental.pallas.tpu as pltpu

BF16, F32 = jnp.bfloat16, jnp.float32
_NT = (((1,), (1,)), ((), ()))


class _Stream:
    def __init__(self, sems, ahead):
        self.sems, self.ahead = sems, ahead
        self.ring = [s.shape[0] for s in sems]
        self.steps = []
        self.started = [0, 0]
        self.done = [0, 0]

    def add(self, *pair):
        i = len(self.steps)
        self.steps.append(tuple(
            pltpu.make_async_copy(src, dst, self.sems[q].at[i % self.ring[q]])
            for q, (src, dst) in enumerate(pair)))
        return i + 1

    def _wait(self, q, n):
        while self.done[q] < n:
            assert self.done[q] < self.started[q]
            self.steps[self.done[q]][q].wait()
            self.done[q] += 1

    def _start(self, q, n):
        while self.started[q] < min(n, len(self.steps)):
            i = self.started[q]
            self._wait(q, i + 1 - self.ring[q])
            self.steps[i][q].start(priority=q)
            self.started[q] += 1

    def start(self):
        for i in range(1, max(self.ahead) + 1):
            for q in (1, 0):
                self._start(q, min(i, self.ahead[q]))

    def _pace(self, n):
        while self.done[1] < min(n, len(self.steps)):
            t = self.done[1] + 1
            self._wait(1, t)
            for q in (0, 1):
                self._start(q, t + self.ahead[q])

    def advance(self, k):
        self._pace(self.done[1] + k)

    def need(self, n, lag=0):
        self._pace(n + lag)
        self._start(0, n)
        self._wait(0, n)

    def finished(self):
        return self.done == [len(self.steps)] * 2


@jax.jit
def pallas_parallel_sum__sliding_block_cached__dense_activation_mish__decode_kernel(
    A_x: jax.Array,
    A_k_cache: jax.Array,
    A_v_cache: jax.Array,
    A_wq: jax.Array,
    A_wo: jax.Array,
    B_x: jax.Array,
    B_w1: jax.Array,
    B_b1: jax.Array,
    B_w2: jax.Array,
):
    del B_x
    B, Sq, D = A_x.shape
    _, Hkv, Sk, Dh = A_k_cache.shape
    Hq = A_wq.shape[1] // Dh
    rep = Hq // Hkv
    W = min(4096, max(256, Sk // 4))
    F = B_w1.shape[1]
    assert (B, Sq, Hkv, rep, Dh) == (2, 1, 8, 4, 128) and W % 256 == 0
    GW = rep * Dh
    scale = Dh ** -0.5
    kv_rows = 128
    kc = 256
    ahead = (12, 48)
    ring0 = 32
    lag = 12
    tail = (2, 1, 1)

    def kernel(x_h, k_h, v_h, wq_h, wo_h, w1_h, b1_h, w2_h, o_ref,
               x_v, b1_v, k_v, v_v, wq_v, wo_v, w1_v, w2_v, s_v, sem_s, sem0, sem1):
        st = _Stream((sem0, sem1), ahead)
        cx = pltpu.make_async_copy(x_h, x_v, sem_s.at[0])
        cb1 = pltpu.make_async_copy(b1_h, b1_v, sem_s.at[1])

        def rows(src, dst, i, r):
            return src.at[pl.ds(i, r)], dst.at[pl.ds(i, r)]

        def split(pieces, ways):
            m = len(pieces) // ways
            assert m * ways == len(pieces)
            return [pieces[j * m:(j + 1) * m] for j in range(ways)]

        def add_interleaved(streams):
            order = [s[i] for i in range(max(map(len, streams))) for s in streams if i < len(s)]
            assert len(order) % 2 == 0
            for pair in zip(order[0::2], order[1::2]):
                n = st.add(*pair)
            return n

        def add_cache(src, dst):
            ends = {}
            for i in range(0, W, kv_rows):
                for g in range(Hkv):
                    ends[i + kv_rows] = st.add(*[
                        (src.at[b, g, pl.ds(Sk - W + i, kv_rows)], dst.at[b, g, pl.ds(i, kv_rows)])
                        for b in range(B)])
            return ends

        half = Hq * Dh // 2
        e_w = add_interleaved(
            split([(wq_h.at[pl.ds(i, 8), pl.ds(c, half)], wq_v.at[pl.ds(i, 8), pl.ds(c, half)])
                   for i in range(0, D, 8) for c in (0, half)], 4)
            + split([rows(w1_h, w1_v, i, 8) for i in range(0, D, 8)], 2)
            + split([rows(w2_h, w2_v, i, 32) for i in range(0, F, 32)], 2))
        e_k = add_cache(k_h, k_v)
        e_v = add_cache(v_h, v_v)
        e_wo = {}
        for j in range(rep):
            pieces = [(g, i) for i in range(0, Dh, 32) for g in range(0, Hkv, 2)]
            if j == rep - 1:
                pieces.sort()
            for g, i in pieces:
                e_wo[j, g] = st.add(*[rows(wo_h, wo_v, (g + q) * GW + j * Dh + i, 32) for q in (0, 1)])

        cx.start()
        cb1.start()
        st.start()

        row = lax.broadcasted_iota(jnp.int32, (8, Dh), 0)
        row_d = lax.broadcasted_iota(jnp.int32, (8, D), 0)
        row_c = lax.broadcasted_iota(jnp.int32, (8, kc), 0)

        cx.wait()
        x = x_v[...].astype(F32)
        xc = x - jnp.mean(x, axis=-1, keepdims=True)
        var = jnp.mean(xc * xc, axis=-1, keepdims=True)
        xn = xc / jnp.sqrt(var + 1e-5)
        xn8 = jnp.where(row_d < rep, xn[0:1, :], xn[1:2, :]).astype(BF16)

        st.need(e_w, lag)
        qs = []
        for g in range(Hkv):
            qf = jnp.dot(xn8, wq_v[:, g * GW:(g + 1) * GW], preferred_element_type=F32)
            qg = qf[:, :Dh]
            for j in range(1, rep):
                qg = jnp.where(row % rep == j, qf[:, j * Dh:(j + 1) * Dh], qg)
            qs.append(qg.astype(BF16))
            st.advance(3)

        cb1.wait()
        b1 = b1_v[...].astype(F32)
        cols = [(c, min(512, F - c)) for c in range(0, F, 512)]
        acts = []
        for c, n in cols:
            h = jnp.dot(xn8, w1_v[:, c:c + n], preferred_element_type=F32)
            h = h + jnp.concatenate([b1[j:j + 1, :] for j in range(c // 128, (c + n) // 128)], axis=1)
            sp = jnp.log1p(jnp.exp(-jnp.abs(h))) + jnp.where(h > 0, h, 0.0)
            acts.append((h * jnp.tanh(sp)).astype(BF16))
            st.advance(3)
        acc = jnp.where(row_d < rep, x[0:1, :], x[1:2, :])
        for (c, n), act in zip(cols, acts):
            acc = acc + jnp.dot(act, w2_v[c:c + n, :], preferred_element_type=F32)
            st.advance(3)

        mx = [None] * Hkv
        for c in range(0, W, kc):
            st.need(e_k[c + kc], lag)
            for g in range(Hkv):
                t = [lax.dot_general(qs[g], k_v[b, g, c:c + kc, :], _NT, preferred_element_type=F32)
                     for b in range(B)]
                s = jnp.where(row_c < rep, t[0], t[1]) * scale
                s_v[g, :, c:c + kc] = s
                for i in range(0, kc, 128):
                    si = s[:, i:i + 128]
                    mx[g] = si if mx[g] is None else jnp.maximum(mx[g], si)
        mx = [jnp.max(t, axis=-1, keepdims=True) for t in mx]

        denom = [None] * Hkv
        o = [None] * Hkv
        for c in range(0, W, kc):
            st.need(e_v[c + kc], lag)
            for g in range(Hkv):
                p = jnp.exp(s_v[g, :, c:c + kc] - mx[g])
                for i in range(0, kc, 128):
                    pi = p[:, i:i + 128]
                    denom[g] = pi if denom[g] is None else denom[g] + pi
                p = p.astype(BF16)
                t = [jnp.dot(p, v_v[b, g, c:c + kc, :], preferred_element_type=F32) for b in range(B)]
                t = jnp.where(row < rep, t[0], t[1])
                o[g] = t if o[g] is None else o[g] + t
        outs = {}
        for g in range(Hkv):
            og = o[g] / jnp.sum(denom[g], axis=-1, keepdims=True)
            for j in range(rep):
                outs[j, g] = jnp.where(row < rep, og[j:j + 1, :], og[rep + j:rep + j + 1, :]).astype(BF16)

        def proj(j, g):
            r = g * GW + j * Dh
            return jnp.dot(outs[j, g], wo_v[r:r + Dh, :], preferred_element_type=F32)

        for j in range(rep - 1):
            st.need(e_wo[j, Hkv - 2])
            for g in range(Hkv):
                acc = acc + proj(j, g)
        g0 = 0
        for n in tail:
            g1 = g0 + 2 * n
            st.need(e_wo[rep - 1, g1 - 2])
            for g in range(g0, g1):
                acc = acc + proj(rep - 1, g)
            g0 = g1
        assert g0 == Hkv and st.finished()
        row_b = lax.broadcasted_iota(jnp.int32, (B, D), 0)
        o_ref[...] = jnp.where(row_b == 0, acc[0:1, :], acc[rep:rep + 1, :]).astype(o_ref.dtype)

    hbm = pl.BlockSpec(memory_space=pltpu.HBM)
    out = pl.pallas_call(
        kernel,
        out_shape=jax.ShapeDtypeStruct((B * Sq, D), A_x.dtype),
        in_specs=[hbm] * 8,
        out_specs=pl.BlockSpec(memory_space=pltpu.VMEM),
        scratch_shapes=[
            pltpu.VMEM((B * Sq, D), A_x.dtype),
            pltpu.VMEM((F // 128, 128), B_b1.dtype),
            pltpu.VMEM((B, Hkv, W, Dh), A_k_cache.dtype),
            pltpu.VMEM((B, Hkv, W, Dh), A_v_cache.dtype),
            pltpu.VMEM(A_wq.shape, A_wq.dtype),
            pltpu.VMEM(A_wo.shape, A_wo.dtype),
            pltpu.VMEM(B_w1.shape, B_w1.dtype),
            pltpu.VMEM(B_w2.shape, B_w2.dtype),
            pltpu.VMEM((Hkv, 8, W), F32),
            pltpu.SemaphoreType.DMA((2,)),
            pltpu.SemaphoreType.DMA((ring0,)),
            pltpu.SemaphoreType.DMA((ahead[1],)),
        ],
        compiler_params=pltpu.CompilerParams(
            vmem_limit_bytes=64 << 20,
            disable_semaphore_checks=True,
            disable_bounds_checks=True,
        ),
    )(A_x.reshape(B * Sq, D), A_k_cache, A_v_cache, A_wq, A_wo, B_w1,
      B_b1.reshape(F // 128, 128), B_w2)
    return out.reshape(B, Sq, D)
```
